```python
import jax
import jax.numpy as jnp

def _softmax(x, axis=-1):
    return jax.nn.softmax(x, axis=axis)

def _gelu(x):
    return jax.nn.gelu(x, approximate=True)

def _silu(x):
    return jax.nn.silu(x)

def _sigmoid(x):
    return jax.nn.sigmoid(x)

def _layernorm(x, axis=-1, eps=1e-05):
    m = jnp.mean(x, axis=axis, keepdims=True)
    v = jnp.var(x, axis=axis, keepdims=True)
    return (x - m) / jnp.sqrt(v + eps)

def _scatter_add(tgt, idx, src, axis=0):
    return tgt.at[idx].add(src)

def _segment_sum(src, seg, n):
    return jax.ops.segment_sum(src, seg, n)

class _Rng:

    def __init__(self, key):
        self._k = key

    def _next(self):
        self._k, sub = jax.random.split(self._k)
        return sub

    def normal(self, shape):
        return jax.random.normal(self._next(), shape, dtype=jnp.bfloat16)

    def randint(self, lo, hi, shape):
        return jax.random.randint(self._next(), shape, lo, hi, dtype=jnp.int32)

    def uniform(self, shape, lo=0.0, hi=1.0):
        return jax.random.uniform(self._next(), shape, jnp.bfloat16, lo, hi)

    def permutation(self, n):
        return jax.random.permutation(self._next(), n)
kernel_name = 'adaLN_cond__ssm_conv_h3__glu_gated_reglu__prompt'

def setup_inputs():
    _rng = _Rng(jax.random.key(int.from_bytes(__import__("os").urandom(4), "little")))
    _w = lambda a: (lambda t: t.astype(jnp.bfloat16) if jnp.issubdtype(t.dtype, jnp.floating) else t)(jnp.asarray(a))

    def _A_setup():
        B, S, D = (1, 2048, 640)
        ks = 4
        return {'q': _w((lambda *s: _rng.normal(s) * 0.05)(B, S, D)), 'k': _w((lambda *s: _rng.normal(s) * 0.05)(B, S, D)), 'v': _w((lambda *s: _rng.normal(s) * 0.05)(B, S, D)), 'shift_k': _w((lambda *s: _rng.normal(s) * 0.05)(D, ks) * 0.5), 'ssm_k': _w((lambda *s: _rng.normal(s) * 0.05)(D, S) * (1.0 / S ** 0.5)), 'ssm_D': _w((lambda *s: _rng.normal(s) * 0.05)(D))}
    _A_in = _A_setup()

    def _B_setup():
        B, S, D, F = (1, 2048, 640, 1536)
        return {'x': _w((lambda *s: _rng.normal(s) * 0.05)(B, S, D)), 'W_gate': _w((lambda *s: _rng.normal(s) * 0.05)(D, F) * (2.0 / D) ** 0.5), 'W_up': _w((lambda *s: _rng.normal(s) * 0.05)(D, F) * (2.0 / D) ** 0.5), 'W_down': _w((lambda *s: _rng.normal(s) * 0.05)(F, D) * (1.0 / F) ** 0.5)}
    _B_in = _B_setup()
    return {'A_q': _A_in['q'], 'A_k': _A_in['k'], 'A_v': _A_in['v'], 'A_shift_k': _A_in['shift_k'], 'A_ssm_k': _A_in['ssm_k'], 'A_ssm_D': _A_in['ssm_D'], 'B_x': _B_in['x'], 'B_W_gate': _B_in['W_gate'], 'B_W_up': _B_in['W_up'], 'B_W_down': _B_in['W_down'], 'c': _w((lambda *s: _rng.normal(s) * 0.05)(1, 640)), 'w_mod': _w((lambda *s: _rng.normal(s) * 0.05)(640, 6 * 640) * 640 ** (-0.5))}

def reference(A_q, A_k, A_v, A_shift_k, A_ssm_k, A_ssm_D, B_x, B_W_gate, B_W_up, B_W_down, c, w_mod):

    def _A_ref(q, k, v, shift_k, ssm_k, ssm_D):
        B, S, D = q.shape
        ks = shift_k.shape[-1]
        k_pad = jnp.pad(k, ((0, 0), (ks - 1, 0), (0, 0)))
        k_shift = jnp.zeros_like(k)
        for t in range(ks):
            k_shift = k_shift + k_pad[:, t:t + S, :] * shift_k[:, ks - 1 - t][None, None, :]
        kv = k_shift * v
        L = 2 * S
        kv_pad = jnp.pad(kv, ((0, 0), (0, S), (0, 0)))
        kf_pad = jnp.pad(ssm_k, ((0, 0), (0, S)))
        kv_f = (lambda x, axes=(-2, -1): jnp.fft.rfft2(x.astype(jnp.float32), axes=axes))(kv_pad[:, None, :, :], axes=(1, 2))
        kf_f = (lambda x, axes=(-2, -1): jnp.fft.rfft2(x.astype(jnp.float32), axes=axes))(kf_pad[:, None, :], axes=(1, 2))
        kf_f = (lambda x, *d: x.transpose(*d))(kf_f, 1, 2, 0)
        y_f = kv_f * kf_f[None, :, :, :]
        y = (lambda x, s, axes=(-2, -1): jnp.fft.irfft2(x, s=s, axes=axes).astype(jnp.bfloat16))(y_f, (1, L), axes=(1, 2))[:, 0, :S, :]
        y = y + kv * ssm_D[None, None, :]
        return q * y

    def _B_ref(x, W_gate, W_up, W_down):
        gate = jnp.einsum('bsd,df->bsf', x, W_gate)
        up = jnp.einsum('bsd,df->bsf', x, W_up)
        gate = gate * (lambda x, dt: x.astype(dt))(gate > 0, gate.dtype)
        h = gate * up
        return jnp.einsum('bsf,fd->bsd', h, W_down)
    x = A_q
    mod = (_silu(c) @ w_mod).reshape(c.shape[0], 6, 1, -1)
    sa, ca, ga, sb, cb, gb = (mod[:, 0].copy(), mod[:, 1].copy(), mod[:, 2].copy(), mod[:, 3].copy(), mod[:, 4].copy(), mod[:, 5].copy())
    h = _layernorm(x, axis=-1) * (1 + ca) + sa
    x = x + ga * _A_ref(h, A_k, A_v, A_shift_k, A_ssm_k, A_ssm_D)
    h = _layernorm(x, axis=-1) * (1 + cb) + sb
    x = x + gb * _B_ref(h, B_W_gate, B_W_up, B_W_down)
    return x
```

```python
import numpy as np
import jax
import jax.numpy as jnp
from jax import lax
import jax.experimental.pallas as pl
import jax.experimental.pallas.tpu as pltpu

OPT = dict(inv=[6, 7], inv1=[8, 9], rho=22, tsum=1, opq='', splitlast=1,
           bars=[[3, 0], [4, 0], [5, 0], [6, 0]],
           pairs=[[2, 1, 3], [3, 1, 9], [4, 2, 0], [5, 3, 0], [6, 4, 0], [7, 5, 0]])

S, D, FF = 2048, 640, 1536
L0 = 128
NC = S // L0
ND = D // 128
RB = 256
NB = S // RB
FB = 512
NF = FF // FB
EPS = 1e-5
I32 = jnp.int32
NSEM = 15 + len(OPT.get('wdg', [[0, 2], [2, 5]]))
NPH = OPT.get('nph', 2)


def _dft_mats():
    n = np.arange(L0, dtype=np.float64)
    m = np.arange(L0, dtype=np.float64)
    w = np.pi * (4 * m + 1) / (2 * L0)
    ang = w[:, None] * n[None, :]
    fr, fi = np.cos(ang), -np.sin(ang)
    F = np.empty((L0 // 8, 2, 8, L0))
    F[:, 0] = fr.reshape(L0 // 8, 8, L0)
    F[:, 1] = fi.reshape(L0 // 8, 8, L0)
    F = F.reshape(2 * L0, L0)
    G = np.empty((L0, L0 // 8, 8, 2))
    G[..., 0] = fr.T.reshape(L0, L0 // 8, 8) / L0
    G[..., 1] = fi.T.reshape(L0, L0 // 8, 8) / L0
    G = G.reshape(L0, 2 * L0)
    return (F.astype(np.float32).astype(jnp.bfloat16),
            G.astype(np.float32).astype(jnp.bfloat16))


_FB, _GB = _dft_mats()

_DUR = [1280] * 6 + [768] * 5
_CUM = np.concatenate([[0], np.cumsum(_DUR)])
_STEP = int(_CUM[-1])


def _ln(x):
    m = jnp.mean(x, axis=-1, keepdims=True)
    xc = x - m
    v = jnp.mean(xc * xc, axis=-1, keepdims=True)
    return xc * lax.rsqrt(v + EPS)


def _kernel(c_hbm, sk_hbm, sd_hbm, x_hbm, k_hbm, v_hbm, ssmk_hbm, wg_hbm, wu_hbm, wd_hbm,
            wmod_hbm, f_hbm, g_hbm, o_hbm,
            cb_, skb, sdb, xb, kb, vb, ssmk, wg, wu, wd, wmod, fm, gm,
            kvb, uf, kf, wf, zs, h2b, x1b, actb, modb, ob, pb, sems, osem, bsem):
    f32, bf16 = jnp.float32, jnp.bfloat16
    nsem = [0]

    def cp(src, dst):
        return (src, dst)

    def group(pairs):
        sem = sems.at[nsem[0]]
        nsem[0] += 1
        return [pltpu.make_async_copy(src, dst, sem) for src, dst in pairs]

    def rows(src, dst, lo, n):
        return cp(src.at[pl.ds(lo, n), :], dst.at[pl.ds(lo, n), :])

    def cols(src, dst, lo, n):
        return cp(src.at[:, pl.ds(lo, n)], dst.at[:, pl.ds(lo, n)])

    c_small = group([cp(f_hbm, fm), cp(c_hbm, cb_), cp(sk_hbm, skb), cp(sd_hbm, sdb), cp(g_hbm, gm)])

    def inputs(blocks):
        return group([cpy for b in blocks for cpy in (
            cols(ssmk_hbm, ssmk, b * RB, RB), rows(k_hbm, kb, b * RB, RB),
            rows(v_hbm, vb, b * RB, RB), rows(x_hbm, xb, b * RB, RB))])
    c_in = {0: inputs([0]), 1: inputs([1]), 2: inputs([2]), 3: inputs([3]), 4: inputs([4, 5, 6, 7])}
    c_wmod = [group([cp(wmod_hbm.at[pl.ds(i * 128, 128), pl.ds(0, 5 * D)], wmod.at[pl.ds(i * 128, 128), pl.ds(0, 5 * D)])])
              for i in range(ND)]
    c_gb = group([cols(wmod_hbm, wmod, 5 * D, D)])
    c_wgu = [group([cols(wg_hbm, wg, j * FB, FB), cols(wu_hbm, wu, j * FB, FB)]) for j in range(NF)]
    c_wd = [group([cols(wd_hbm, wd, n * 128, 128) for n in range(n0, n1)]) for n0, n1 in OPT.get('wdg', [[0, 2], [2, 5]])]

    order = (c_small + c_in[0] + c_in[1] + sum(c_wmod, []) + sum(c_wgu, []) + sum(c_wd, [])
             + c_in[2] + c_gb + c_in[3] + c_in[4])
    assert nsem[0] == NSEM, nsem[0]
    for cpy in order:
        cpy.start()

    nmark = [0]

    def mark(name):
        if OPT.get('scopes'):
            with jax.named_scope('M%02d_%s' % (nmark[0], name)):
                modb[0:1, 0:128] = jnp.zeros((1, 128), f32)
            nmark[0] += 1

    def W(cs):
        def go():
            for cpy in cs:
                cpy.wait()
            mark('wait')
        return go

    dot = lambda a, b: jnp.dot(a, b, preferred_element_type=f32)
    state = {}
    tok32 = lambda x: pltpu.bitcast(x, I32)
    OPQ = OPT.get('opq', 'uk')
    zst = lambda: state['z0'] if 'u' in OPQ else 0
    zld = lambda: state['z1'] if 'u' in OPQ else 0
    zst2 = lambda: state['z0'] if 'w' in OPQ else 0
    zld2 = lambda: state['z1'] if 'w' in OPQ else 0

    def FK(c):
        def go():
            r = lax.dot_general(fm[...], ssmk[:, c * L0:(c + 1) * L0], (((1,), (1,)), ((), ())),
                                preferred_element_type=f32)
            for dt in range(ND):
                kf[dt + zst(), c] = r[:, dt * 128:(dt + 1) * 128]
        return go

    def KVgen(j):
        sk = skb[...].astype(f32)
        r0 = j * L0
        kc = kb[r0:r0 + L0, :].astype(f32)
        if j == 0:
            prev = jnp.zeros((8, D), f32)
        else:
            prev = kb[r0 - 16:r0, :].astype(f32)[8:, :]
        ext = jnp.concatenate([prev, kc], axis=0)
        acc = kc * sk[0:1, :]
        for t in range(1, 4):
            acc = acc + pltpu.roll(ext, t, axis=0)[8:, :] * sk[t:t + 1, :]
        kv = (acc * vb[r0:r0 + L0, :].astype(f32)).astype(bf16)
        kv = pltpu.bitcast(kv, I32)
        kvb[r0 // 2:(r0 + L0) // 2, :] = kv
        for g in range(L0 // 16):
            for dt in range(ND):
                yield kv[g * 8:(g + 1) * 8, dt * 128:(dt + 1) * 128]

    def SD(j):
        def go():
            r = dot(fm[...], pltpu.bitcast(kvb[j * L0 // 2:(j + 1) * L0 // 2, :], bf16))
            for dt in range(ND):
                uf[dt + zst(), j] = r[:, dt * 128:(dt + 1) * 128]
        return go

    def CVtile(b, t):
        dt, ft = t // 16, t % 16
        re = slice(ft * 16, ft * 16 + 8)
        im = slice(ft * 16 + 8, ft * 16 + 16)
        both = slice(ft * 16, ft * 16 + 16)
        a0, a1 = 2 * b, 2 * b + 1
        gauss = OPT.get('gauss', 0)
        z = [None, None]

        def ldu(j):
            ur, ui = uf[dt + zld(), j, re, :], uf[dt + zld(), j, im, :]
            return (ur, ui, ur + ui) if gauss else (ur, ui)
        ulast = ldu(a1)

        def mac(zz, kk, uu):
            if gauss:
                p = (kk[0] * uu[0], kk[1] * uu[1], kk[2] * uu[2])
            elif OPT.get('chain2') and zz is not None:
                return ((zz[0] + kk[0] * uu[0]) - kk[1] * uu[1], (zz[1] + kk[0] * uu[1]) + kk[1] * uu[0])
            else:
                p = (kk[0] * uu[0] - kk[1] * uu[1], kk[0] * uu[1] + kk[1] * uu[0])
            if zz is None:
                return p
            return tuple(x + y for x, y in zip(zz, p))

        def fin(zz):
            if gauss:
                return (zz[0] - zz[1], zz[2] - zz[0] - zz[1])
            return zz
        n = a1 + 1
        nph = NPH if n >= 6 else 1
        bounds = [int(round((i + 1) * n / nph)) - 1 for i in range(nph - 1)]
        for c in range(n):
            kr, ki = kf[dt + zld(), c, re, :], kf[dt + zld(), c, im, :]
            kk = (kr, ki, kr + ki) if gauss else (kr, ki)
            z[1] = mac(z[1], kk, ulast)
            if c <= a0:
                if c < a0 or not gauss:
                    ulast = ldu(a0 - c)
                    z[0] = mac(z[0], kk, ulast)
                else:
                    ulast = (uf[dt + zld(), 0, re, :], uf[dt + zld(), 0, im, :])
                    ulast = (ulast[0], ulast[1], ulast[0] + ulast[1])
                    z[0] = mac(z[0], kk, ulast)
            if c in bounds:
                ts = OPT.get('tsum', 1)
                if ts == 1:
                    tot = z[1][0] + z[1][1]
                    for x in z[1][2:] + z[0]:
                        tot = tot + x
                    yield tok32(tot)
                elif ts == 4:
                    yield tok32(z[1][0])
                    yield tok32(z[0][1])
                    yield tok32(z[1][1])
                    yield tok32(z[0][0])
                else:
                    yield tok32(z[1][0])
        z = [fin(z[0]), fin(z[1])]
        if b == 0:
            w0r, w0i = z[0]
        else:
            w0r = z[0][0] - zs[dt + zld2(), im, :]
            w0i = z[0][1] + zs[dt + zld2(), re, :]
        w1r = z[1][0] - z[0][1]
        w1i = z[1][1] + z[0][0]
        if b < NB - 1:
            zs[dt + zst2(), re, :] = z[1][0]
            zs[dt + zst2(), im, :] = z[1][1]
        w0 = pltpu.pack_elementwise([w0r, w0i], packed_dtype=bf16)
        w1 = pltpu.pack_elementwise([w1r, w1i], packed_dtype=bf16)
        rr = slice(ft * 8, ft * 8 + 8)
        wf[dt + zst2(), a0, rr, :] = w0
        wf[dt + zst2(), a1, rr, :] = w1
        yield (w0 | w1) if OPT.get('tsum', 1) else tok32(w1r)

    def CVgen(b, lo=0, hi=80):
        for t in range(lo, hi):
            yield from CVtile(b, t)

    def ncv(b, nt=80):
        if 2 * b + 2 < 6:
            return nt
        return nt * (1 + (NPH - 1) * {3: 2, 4: 4}.get(OPT.get('tsum', 1), 1))

    def MOD(i):
        def go():
            if i == 0:
                cc = cb_[...].astype(f32)
                state['sc'] = jnp.broadcast_to((cc * jax.nn.sigmoid(cc)).astype(bf16), (16, D))
            p = dot(state['sc'][:, i * 128:(i + 1) * 128], wmod[i * 128:(i + 1) * 128, 0:5 * D])[0:8, :]
            state['mod'] = p if i == 0 else state['mod'] + p
        return go

    def MODfin():
        m = state['mod'][0:1, :]
        state['sa'] = m[:, 0:D]
        state['ca1'] = 1.0 + m[:, D:2 * D]
        state['ga'] = m[:, 2 * D:3 * D]
        state['sb'] = m[:, 3 * D:4 * D]
        state['cb1'] = 1.0 + m[:, 4 * D:5 * D]
        state['sd'] = sdb[...].astype(f32).reshape(1, D)

    def MODgb():
        state['gb'] = dot(state['sc'], wmod[:, 5 * D:6 * D])[0:1, :]

    ys = {}

    def INV(a):
        def go():
            w = jnp.concatenate([pltpu.bitcast(wf[dt + zld2(), a], bf16) for dt in range(ND)], axis=1)
            ys[a] = dot(gm[...], w)
        return go

    def GATEgen(a):
        r0 = a * L0
        y = ys[a]
        x = xb[r0:r0 + L0, :].astype(f32)
        kv = pltpu.bitcast(kvb[r0 // 2:(r0 + L0) // 2, :], bf16).astype(f32)
        h = _ln(x) * state['ca1'] + state['sa']
        x1 = x + state['ga'] * (h * (y + kv * state['sd']))
        x1b[r0:r0 + L0, :] = x1
        h2 = (_ln(x1) * state['cb1'] + state['sb']).astype(bf16)
        h2 = pltpu.bitcast(h2, I32)
        h2b[r0 // 2:(r0 + L0) // 2, :] = h2
        for g in range(L0 // 16):
            for dt in range(ND):
                yield h2[g * 8:(g + 1) * 8, dt * 128:(dt + 1) * 128]

    def drain(gen):
        def go():
            for _ in gen():
                pass
        return go

    def out_copy(s):
        return pltpu.make_async_copy(ob.at[pl.ds(s * RB, RB), :], o_hbm.at[pl.ds(s * RB, RB), :], osem)

    SPLIT_LAST = OPT.get('splitlast', 0)

    def last_copy(n):
        r = pl.ds((NB - 1) * RB, RB)
        cs = pl.ds(n * 128, 128)
        return pltpu.make_async_copy(ob.at[r, cs], o_hbm.at[r, cs], osem)

    def BAR():
        pl.semaphore_signal(bsem, 1)
        pl.semaphore_wait(bsem, 1)

    def FIN0():
        MODgb()
        ob[0:RB, :] = (x1b[0:RB, :] + state['gb'] * pb[...]).astype(bf16)
        out_copy(0).start()

    streams = []
    pre = {}

    def T(s, d):
        return s * _STEP + float(np.interp(d, np.arange(12), _CUM))

    def stream(t_lo, t_hi, ntok, gen):
        streams.append(dict(lo=t_lo, hi=t_hi, n=ntok, gen=gen, it=None, done=0))

    def before(s, d, *fns):
        pre.setdefault((s, d), []).extend(fns)

    _planC(OPT, stream, before, T, dict(
        W=W, FK=FK, SD=SD, INV=INV, KV=lambda j: (lambda: KVgen(j)),
        CV=lambda b, lo=0, hi=80: (lambda: CVgen(b, lo, hi)), GATE=lambda a: (lambda: GATEgen(a)),
        ncv=ncv, drain=drain, MODgb=MODgb, FIN0=FIN0, BAR=BAR,
        c_in=c_in, c_wgu=c_wgu, c_wd=c_wd, c_gb=c_gb))

    def next_token(t):
        best = None
        for st in streams:
            if st['done'] >= st['n']:
                continue
            target = st['lo'] + (st['done'] + 1) * (st['hi'] - st['lo']) / st['n']
            if target <= t + 1e-6 and (best is None or target < best[0]):
                best = (target, st)
        if best is None:
            return None
        st = best[1]
        if st['it'] is None:
            st['it'] = st['gen']()
        tok = next(st['it'])
        st['done'] += 1
        if st['done'] == st['n']:
            for _ in st['it']:
                raise AssertionError('stream has more tokens than planned')
        return tok

    def tie(wref, nr, c0, nc, t0, t1):
        nslot = (nr // 16) * (nc // 128)
        i = 0
        rws = []
        for kt in range(nr // 128):
            cls = []
            for nt in range(nc // 128):
                pcs = []
                for r in range(8):
                    i += 1
                    w = wref[kt * 128 + r * 16:kt * 128 + (r + 1) * 16, c0 + nt * 128:c0 + (nt + 1) * 128]
                    tok = next_token(t0 + (t1 - t0) * i / nslot)
                    if tok is not None:
                        w = pltpu.bitcast(jnp.where(state['never'], tok, pltpu.bitcast(w, I32)), bf16)
                    pcs.append(w)
                cls.append(jnp.concatenate(pcs, axis=0))
            rws.append(jnp.concatenate(cls, axis=1))
        return jnp.concatenate(rws, axis=0)

    W(c_small)()
    state['never'] = gm[0:16, 0:128].astype(f32)[0:8, :] > 2.0
    gmax = jnp.max(gm[0:16, 0:128].astype(f32))
    state['z0'] = (gmax > 2.0).astype(jnp.int32)
    state['z1'] = (gmax > 3.0).astype(jnp.int32)
    for b in range(2):
        W(c_in[b])()
        FK(2 * b)(); FK(2 * b + 1)()
        drain(lambda: KVgen(2 * b))(); SD(2 * b)()
        drain(lambda: KVgen(2 * b + 1))(); SD(2 * b + 1)()
        drain(lambda: CVgen(b))()
        INV(2 * b)(); INV(2 * b + 1)()
    for i in range(ND):
        W(c_wmod[i])()
        MOD(i)()
    MODfin()
    mark('modfin')
    drain(lambda: GATEgen(0))(); drain(lambda: GATEgen(1))()

    for s in range(NB):
        h2 = lambda: pltpu.bitcast(h2b[s * RB // 2:(s + 1) * RB // 2, :], bf16)
        for j in range(NF):
            for fn in pre.get((s, 2 * j), []):
                fn()
            g = dot(h2(), tie(wg, D, j * FB, FB, T(s, 2 * j), T(s, 2 * j + 1)))
            for fn in pre.get((s, 2 * j + 1), []):
                fn()
            u = dot(h2(), tie(wu, D, j * FB, FB, T(s, 2 * j + 1), T(s, 2 * j + 2)))
            actb[:, j * FB:(j + 1) * FB] = pltpu.bitcast((jnp.maximum(g, 0.0) * u).astype(bf16), I32)
        for n in range(ND):
            for fn in pre.get((s, 6 + n), []):
                fn()
            p = dot(pltpu.bitcast(actb[...], bf16), tie(wd, FF, n * 128, 128, T(s, 6 + n), T(s, 7 + n)))
            if s == 0:
                pb[:, n * 128:(n + 1) * 128] = p
                continue
            ob[s * RB:(s + 1) * RB, n * 128:(n + 1) * 128] = (
                x1b[s * RB:(s + 1) * RB, n * 128:(n + 1) * 128]
                + state['gb'][:, n * 128:(n + 1) * 128] * p).astype(bf16)
            if s == NB - 1 and SPLIT_LAST:
                last_copy(n).start()
        for fn in pre.get((s, 11), []):
            fn()
        if s != 0 and not (s == NB - 1 and SPLIT_LAST):
            out_copy(s).start()
        mark('step%d' % s)
    for st in streams:
        assert st['done'] == st['n'], st
    for s in range(NB - 1 if SPLIT_LAST else NB):
        out_copy(s).wait()
    if SPLIT_LAST:
        for n in range(ND):
            last_copy(n).wait()
    mark('end')


def _planC(opt, stream, before, T, k):
    W, INV, CV, GATE, FK, SD, KV, drain = k['W'], k['INV'], k['CV'], k['GATE'], k['FK'], k['SD'], k['KV'], k['drain']
    ncv, c_in, c_wgu, c_wd, c_gb = k['ncv'], k['c_in'], k['c_wgu'], k['c_wd'], k['c_gb']
    inv = {s: opt.get('inv', [5, 6]) for s in range(NB)}
    inv[1] = opt.get('inv1', [7, 8])
    slack = opt.get('slack', 0.5)

    def pair(b, s, d, wait=None):
        if wait is not None:
            before(s, d, W(wait))
        before(s, d, FK(2 * b), FK(2 * b + 1), drain(KV(2 * b)), SD(2 * b), drain(KV(2 * b + 1)), SD(2 * b + 1))
        rel[b] = T(s, d)
    rel = {}
    before(0, 0, W(c_wgu[0]))
    before(0, opt.get('g23', 1), drain(GATE(2)), drain(GATE(3)))
    before(0, 2, W(c_wgu[1]))
    before(0, 4, W(c_wgu[2]))
    for grp, (n0, n1) in zip(c_wd, opt.get('wdg', [[0, 2], [2, 5]])):
        before(0, 6 + n0, W(grp))
    pos = opt.get('pairs', [[2, 1, 3], [3, 1, 9], [4, 2, 1], [5, 2, 8], [6, 3, 8], [7, 4, 8]])
    for b, s, d in pos:
        wait = c_in[b] + (c_gb if b == 2 else []) if b <= 4 else None
        pair(b, s, d, wait)
        if b == 2:
            before(s, d, k['FIN0'])
    for s in range(1, NB - 1):
        b = s + 1
        before(s, inv[s][0], INV(2 * b), drain(GATE(2 * b)))
        before(s, inv[s][1], INV(2 * b + 1), drain(GATE(2 * b + 1)))

    for s, d in opt.get('bars', []):
        before(s, d, k['BAR'])
    rho = opt.get('rho', 24.0) / T(1, 0)
    t = 0.0
    for b in range(2, NB):
        units = 4 * b + 3
        lo = max(t, rel[b])
        hi = min(lo + units / rho, T(b - 1, inv[b - 1][0] - slack))
        stream(lo, hi, ncv(b), CV(b))
        t = hi


@jax.jit
def pallas_adaLN_cond__ssm_conv_h3__glu_gated_reglu__prompt_kernel(
        A_q, A_k, A_v, A_shift_k, A_ssm_k, A_ssm_D, B_x, B_W_gate, B_W_up, B_W_down, c, w_mod):
    bf16, f32 = jnp.bfloat16, jnp.float32
    any_spec = pl.BlockSpec(memory_space=pl.ANY)
    V = pltpu.VMEM
    out = pl.pallas_call(
        _kernel,
        out_shape=jax.ShapeDtypeStruct((S, D), bf16),
        in_specs=[any_spec] * 13,
        out_specs=any_spec,
        scratch_shapes=[
            V((1, D), bf16), V((4, D), bf16), V((D,), bf16),
            V((S, D), bf16), V((S, D), bf16), V((S, D), bf16),
            V((D, S), bf16),
            V((D, FF), bf16), V((D, FF), bf16), V((FF, D), bf16),
            V((D, 6 * D), bf16),
            V((2 * L0, L0), bf16), V((L0, 2 * L0), bf16),
            V((S // 2, D), I32),
            V((ND, NC, 2 * L0, 128), f32), V((ND, NC, 2 * L0, 128), f32),
            V((ND, NC, L0, 128), I32),
            V((ND, 2 * L0, 128), f32),
            V((S // 2, D), I32), V((S, D), f32), V((RB // 2, FF), I32), V((8, 6 * D), f32), V((S, D), bf16), V((RB, D), f32),
            pltpu.SemaphoreType.DMA((NSEM,)), pltpu.SemaphoreType.DMA, pltpu.SemaphoreType.REGULAR,
        ],
        compiler_params=pltpu.CompilerParams(vmem_limit_bytes=110 * 1024 * 1024,
                                             disable_semaphore_checks=bool(OPT.get('nosemchk', 0)), flags=OPT.get('flags')),
    )(c, A_shift_k.T, A_ssm_D,
      A_q.reshape(S, D), A_k.reshape(S, D), A_v.reshape(S, D), A_ssm_k,
      B_W_gate, B_W_up, B_W_down, w_mod, jnp.asarray(_FB), jnp.asarray(_GB))
    return out.reshape(1, S, D)
```

```python
import numpy as np
import jax
import jax.numpy as jnp
from jax import lax
import jax.experimental.pallas as pl
import jax.experimental.pallas.tpu as pltpu

OPT = dict(inv=[5, 6], inv1=[8, 9], tsum=2, opq='', splitlast=1,
           bars=[[2, 0], [3, 0], [4, 0], [5, 0], [6, 0]], wsplit=1, fin0late=[7, 1],
           pairs=[[2, 1, 3], [3, 1, 9], [4, 2, 0], [5, 3, 0], [6, 4, 0], [7, 5, 0]])

S, D, FF = 2048, 640, 1536
L0 = 128
NC = S // L0
ND = D // 128
RB = 256
NB = S // RB
FB = 512
NF = FF // FB
EPS = 1e-5
I32 = jnp.int32
WSPLIT = OPT.get('wsplit', 0)
NSEM = 16 + 3 * WSPLIT + len(OPT.get('wdg', [[0, 2], [2, 5]]))
NPH = OPT.get('nph', 2)


def _dft_mats():
    n = np.arange(L0, dtype=np.float64)
    m = np.arange(L0, dtype=np.float64)
    w = np.pi * (4 * m + 1) / (2 * L0)
    ang = w[:, None] * n[None, :]
    fr, fi = np.cos(ang), -np.sin(ang)
    F = np.empty((L0 // 8, 2, 8, L0))
    F[:, 0] = fr.reshape(L0 // 8, 8, L0)
    F[:, 1] = fi.reshape(L0 // 8, 8, L0)
    F = F.reshape(2 * L0, L0)
    G = np.empty((L0, L0 // 8, 8, 2))
    G[..., 0] = fr.T.reshape(L0, L0 // 8, 8) / L0
    G[..., 1] = fi.T.reshape(L0, L0 // 8, 8) / L0
    G = G.reshape(L0, 2 * L0)
    return (F.astype(np.float32).astype(jnp.bfloat16),
            G.astype(np.float32).astype(jnp.bfloat16))


_FB, _GB = _dft_mats()

_DUR = [1280] * 6 + [768] * 5
_CUM = np.concatenate([[0], np.cumsum(_DUR)])
_STEP = int(_CUM[-1])


def _ln(x):
    m = jnp.mean(x, axis=-1, keepdims=True)
    xc = x - m
    v = jnp.mean(xc * xc, axis=-1, keepdims=True)
    return xc * lax.rsqrt(v + EPS)


def _kernel(c_hbm, sk_hbm, sd_hbm, x_hbm, k_hbm, v_hbm, ssmk_hbm, wg_hbm, wu_hbm, wd_hbm,
            wmod_hbm, f_hbm, g_hbm, o_hbm,
            cb_, skb, sdb, xb, kb, vb, ssmk, wg, wu, wd, wmod, fm, gm,
            kvb, uf, kf, wf, zs, h2b, x1b, actb, modb, ob, pb, sems, osem, bsem):
    f32, bf16 = jnp.float32, jnp.bfloat16
    nsem = [0]

    def cp(src, dst):
        return (src, dst)

    def group(pairs):
        sem = sems.at[nsem[0]]
        nsem[0] += 1
        return [pltpu.make_async_copy(src, dst, sem) for src, dst in pairs]

    def rows(src, dst, lo, n):
        return cp(src.at[pl.ds(lo, n), :], dst.at[pl.ds(lo, n), :])

    def cols(src, dst, lo, n):
        return cp(src.at[:, pl.ds(lo, n)], dst.at[:, pl.ds(lo, n)])

    c_small = group([cp(f_hbm, fm), cp(c_hbm, cb_), cp(sk_hbm, skb), cp(sd_hbm, sdb), cp(g_hbm, gm)])

    def inputs(blocks):
        return group([cpy for b in blocks for cpy in (
            cols(ssmk_hbm, ssmk, b * RB, RB), rows(k_hbm, kb, b * RB, RB),
            rows(v_hbm, vb, b * RB, RB), rows(x_hbm, xb, b * RB, RB))])
    c_in = {0: inputs([0]), 2: inputs([2]), 3: inputs([3]), 4: inputs([4, 5, 6, 7])}
    c_in[1] = group([cols(ssmk_hbm, ssmk, RB, RB), rows(k_hbm, kb, RB, RB), rows(v_hbm, vb, RB, RB)])
    c_x1 = group([rows(x_hbm, xb, RB, RB)])
    c_wmod = [group([cp(wmod_hbm.at[pl.ds(i * 128, 128), pl.ds(0, 5 * D)], wmod.at[pl.ds(i * 128, 128), pl.ds(0, 5 * D)])])
              for i in range(ND)]
    c_gb = group([cols(wmod_hbm, wmod, 5 * D, D)])
    if WSPLIT:
        c_wgu = [group([cols(w_hbm, w, j * FB, FB)]) for j in range(NF) for w_hbm, w in ((wg_hbm, wg), (wu_hbm, wu))]
    else:
        c_wgu = [group([cols(wg_hbm, wg, j * FB, FB), cols(wu_hbm, wu, j * FB, FB)]) for j in range(NF)]
    c_wd = [group([cols(wd_hbm, wd, n * 128, 128) for n in range(n0, n1)]) for n0, n1 in OPT.get('wdg', [[0, 2], [2, 5]])]

    ORDER1 = OPT.get('order1', 0)
    front = c_in[0] + sum(c_wmod, []) + c_in[1] if ORDER1 else c_in[0] + c_in[1] + sum(c_wmod, [])
    nw = 2 if WSPLIT else 1
    order = (c_small + front + sum(c_wgu[:nw], []) + c_x1 + sum(c_wgu[nw:], []) + sum(c_wd, [])
             + c_in[2] + c_gb + c_in[3] + c_in[4])
    assert nsem[0] == NSEM, nsem[0]
    for cpy in order:
        cpy.start()

    nmark = [0]

    def mark(name):
        if OPT.get('scopes'):
            with jax.named_scope('M%02d_%s' % (nmark[0], name)):
                modb[0:1, 0:128] = jnp.zeros((1, 128), f32)
            nmark[0] += 1

    def W(cs):
        def go():
            for cpy in cs:
                cpy.wait()
            mark('wait')
        return go

    dot = lambda a, b: jnp.dot(a, b, preferred_element_type=f32)
    state = {}
    tok32 = lambda x: pltpu.bitcast(x, I32)
    OPQ = OPT.get('opq', 'uk')
    zst = lambda: state['z0'] if 'u' in OPQ else 0
    zld = lambda: state['z1'] if 'u' in OPQ else 0
    zst2 = lambda: state['z0'] if 'w' in OPQ else 0
    zld2 = lambda: state['z1'] if 'w' in OPQ else 0

    def FK(c):
        def go():
            r = lax.dot_general(fm[...], ssmk[:, c * L0:(c + 1) * L0], (((1,), (1,)), ((), ())),
                                preferred_element_type=f32)
            for dt in range(ND):
                kf[dt + zst(), c] = r[:, dt * 128:(dt + 1) * 128]
        return go

    def KVgen(j):
        sk = skb[...].astype(f32)
        r0 = j * L0
        kc = kb[r0:r0 + L0, :].astype(f32)
        if j == 0:
            prev = jnp.zeros((8, D), f32)
        else:
            prev = kb[r0 - 16:r0, :].astype(f32)[8:, :]
        ext = jnp.concatenate([prev, kc], axis=0)
        acc = kc * sk[0:1, :]
        for t in range(1, 4):
            acc = acc + pltpu.roll(ext, t, axis=0)[8:, :] * sk[t:t + 1, :]
        kv = (acc * vb[r0:r0 + L0, :].astype(f32)).astype(bf16)
        kv = pltpu.bitcast(kv, I32)
        kvb[r0 // 2:(r0 + L0) // 2, :] = kv
        for g in range(L0 // 16):
            for dt in range(ND):
                yield kv[g * 8:(g + 1) * 8, dt * 128:(dt + 1) * 128]

    def SD(j):
        def go():
            r = dot(fm[...], pltpu.bitcast(kvb[j * L0 // 2:(j + 1) * L0 // 2, :], bf16))
            for dt in range(ND):
                uf[dt + zst(), j] = r[:, dt * 128:(dt + 1) * 128]
        return go

    def CVtile(b, t):
        dt, ft = t // 16, t % 16
        re = slice(ft * 16, ft * 16 + 8)
        im = slice(ft * 16 + 8, ft * 16 + 16)
        both = slice(ft * 16, ft * 16 + 16)
        a0, a1 = 2 * b, 2 * b + 1
        gauss = OPT.get('gauss', 0)
        z = [None, None]

        def ldu(j):
            ur, ui = uf[dt + zld(), j, re, :], uf[dt + zld(), j, im, :]
            return (ur, ui, ur + ui) if gauss else (ur, ui)
        ulast = ldu(a1)

        def mac(zz, kk, uu):
            if gauss:
                p = (kk[0] * uu[0], kk[1] * uu[1], kk[2] * uu[2])
            elif OPT.get('chain2') and zz is not None:
                return ((zz[0] + kk[0] * uu[0]) - kk[1] * uu[1], (zz[1] + kk[0] * uu[1]) + kk[1] * uu[0])
            else:
                p = (kk[0] * uu[0] - kk[1] * uu[1], kk[0] * uu[1] + kk[1] * uu[0])
            if zz is None:
                return p
            return tuple(x + y for x, y in zip(zz, p))

        def fin(zz):
            if gauss:
                return (zz[0] - zz[1], zz[2] - zz[0] - zz[1])
            return zz
        n = a1 + 1
        nph = NPH if n >= 6 else 1
        bounds = [int(round((i + 1) * n / nph)) - 1 for i in range(nph - 1)]
        for c in range(n):
            kr, ki = kf[dt + zld(), c, re, :], kf[dt + zld(), c, im, :]
            kk = (kr, ki, kr + ki) if gauss else (kr, ki)
            z[1] = mac(z[1], kk, ulast)
            if c <= a0:
                if c < a0 or not gauss:
                    ulast = ldu(a0 - c)
                    z[0] = mac(z[0], kk, ulast)
                else:
                    ulast = (uf[dt + zld(), 0, re, :], uf[dt + zld(), 0, im, :])
                    ulast = (ulast[0], ulast[1], ulast[0] + ulast[1])
                    z[0] = mac(z[0], kk, ulast)
            if c in bounds:
                ts = OPT.get('tsum', 1)
                if ts == 1:
                    tot = z[1][0] + z[1][1]
                    for x in z[1][2:] + z[0]:
                        tot = tot + x
                    yield tok32(tot)
                elif ts == 4:
                    yield tok32(z[1][0])
                    yield tok32(z[0][1])
                    yield tok32(z[1][1])
                    yield tok32(z[0][0])
                else:
                    yield tok32(z[1][0])
        z = [fin(z[0]), fin(z[1])]
        if b == 0:
            w0r, w0i = z[0]
        else:
            w0r = z[0][0] - zs[dt + zld2(), im, :]
            w0i = z[0][1] + zs[dt + zld2(), re, :]
        w1r = z[1][0] - z[0][1]
        w1i = z[1][1] + z[0][0]
        if b < NB - 1:
            zs[dt + zst2(), re, :] = z[1][0]
            zs[dt + zst2(), im, :] = z[1][1]
        w0 = pltpu.pack_elementwise([w0r, w0i], packed_dtype=bf16)
        w1 = pltpu.pack_elementwise([w1r, w1i], packed_dtype=bf16)
        rr = slice(ft * 8, ft * 8 + 8)
        wf[dt + zst2(), a0, rr, :] = w0
        wf[dt + zst2(), a1, rr, :] = w1
        yield (w0 | w1) if OPT.get('tsum', 1) else tok32(w1r)

    def CVgen(b, lo=0, hi=80):
        for t in range(lo, hi):
            yield from CVtile(b, t)

    def ncv(b, nt=80):
        if 2 * b + 2 < 6:
            return nt
        return nt * (1 + (NPH - 1) * {3: 2, 4: 4}.get(OPT.get('tsum', 1), 1))

    def MOD(i):
        def go():
            if i == 0:
                cc = cb_[...].astype(f32)
                state['sc'] = jnp.broadcast_to((cc * jax.nn.sigmoid(cc)).astype(bf16), (16, D))
            p = dot(state['sc'][:, i * 128:(i + 1) * 128], wmod[i * 128:(i + 1) * 128, 0:5 * D])[0:8, :]
            state['mod'] = p if i == 0 else state['mod'] + p
        return go

    def MODfin():
        m = state['mod'][0:1, :]
        state['sa'] = m[:, 0:D]
        state['ca1'] = 1.0 + m[:, D:2 * D]
        state['ga'] = m[:, 2 * D:3 * D]
        state['sb'] = m[:, 3 * D:4 * D]
        state['cb1'] = 1.0 + m[:, 4 * D:5 * D]

    def MODgb():
        state['gb'] = dot(state['sc'], wmod[:, 5 * D:6 * D])[0:1, :]

    ys = {}

    def INV(a):
        def go():
            w = jnp.concatenate([pltpu.bitcast(wf[dt + zld2(), a], bf16) for dt in range(ND)], axis=1)
            ys[a] = dot(gm[...], w)
        return go

    gpre = {}

    def GPRE(a):
        r0 = a * L0
        x = xb[r0:r0 + L0, :].astype(f32)
        kv = pltpu.bitcast(kvb[r0 // 2:(r0 + L0) // 2, :], bf16).astype(f32)
        gpre[a] = (x, _ln(x), ys[a] + kv * state['sd'])

    def GATEgen(a):
        r0 = a * L0
        if a not in gpre:
            GPRE(a)
        x, xn, t = gpre.pop(a)
        h = xn * state['ca1'] + state['sa']
        x1 = x + state['ga'] * (h * t)
        x1b[r0:r0 + L0, :] = x1
        h2 = (_ln(x1) * state['cb1'] + state['sb']).astype(bf16)
        h2 = pltpu.bitcast(h2, I32)
        h2b[r0 // 2:(r0 + L0) // 2, :] = h2
        for g in range(L0 // 16):
            for dt in range(ND):
                yield h2[g * 8:(g + 1) * 8, dt * 128:(dt + 1) * 128]

    def drain(gen):
        def go():
            for _ in gen():
                pass
        return go

    def out_copy(s):
        return pltpu.make_async_copy(ob.at[pl.ds(s * RB, RB), :], o_hbm.at[pl.ds(s * RB, RB), :], osem)

    SPLIT_LAST = OPT.get('splitlast', 0)

    def last_copy(n):
        r = pl.ds((NB - 1) * RB, RB)
        cs = pl.ds(n * 128, 128)
        return pltpu.make_async_copy(ob.at[r, cs], o_hbm.at[r, cs], osem)

    def BAR():
        pl.semaphore_signal(bsem, 1)
        pl.semaphore_wait(bsem, 1)

    def FIN0():
        MODgb()
        if not OPT.get('fin0late'):
            FIN0b()

    def FIN0b():
        ob[0:RB, :] = (x1b[0:RB, :] + state['gb'] * pb[...]).astype(bf16)
        out_copy(0).start()

    streams = []
    pre = {}

    def T(s, d):
        return s * _STEP + float(np.interp(d, np.arange(12), _CUM))

    def stream(targets, gen):
        streams.append(dict(t=targets, n=len(targets), gen=gen, it=None, done=0))

    def before(s, d, *fns):
        pre.setdefault((s, d), []).extend(fns)

    _planC(OPT, stream, before, T, dict(
        W=W, FK=FK, SD=SD, INV=INV, KV=lambda j: (lambda: KVgen(j)),
        CV=lambda b, lo=0, hi=80: (lambda: CVgen(b, lo, hi)), GATE=lambda a: (lambda: GATEgen(a)),
        ncv=ncv, drain=drain, MODgb=MODgb, FIN0=FIN0, FIN0b=FIN0b, BAR=BAR,
        c_in=c_in, c_x1=c_x1, c_wgu=c_wgu, c_wd=c_wd, c_gb=c_gb))

    def next_token(t):
        best = None
        for st in streams:
            if st['done'] >= st['n']:
                continue
            target = st['t'][st['done']]
            if target <= t + 1e-6 and (best is None or target < best[0]):
                best = (target, st)
        if best is None:
            return None
        st = best[1]
        if st['it'] is None:
            st['it'] = st['gen']()
        tok = next(st['it'])
        st['done'] += 1
        if st['done'] == st['n']:
            for _ in st['it']:
                raise AssertionError('stream has more tokens than planned')
        return tok

    def tie(wref, nr, c0, nc, t0, t1):
        nslot = (nr // 16) * (nc // 128)
        i = 0
        rws = []
        for kt in range(nr // 128):
            cls = []
            for nt in range(nc // 128):
                pcs = []
                for r in range(8):
                    i += 1
                    w = wref[kt * 128 + r * 16:kt * 128 + (r + 1) * 16, c0 + nt * 128:c0 + (nt + 1) * 128]
                    tok = next_token(t0 + (t1 - t0) * i / nslot)
                    if tok is not None:
                        w = pltpu.bitcast(jnp.where(state['never'], tok, pltpu.bitcast(w, I32)), bf16)
                    pcs.append(w)
                cls.append(jnp.concatenate(pcs, axis=0))
            rws.append(jnp.concatenate(cls, axis=1))
        return jnp.concatenate(rws, axis=0)

    W(c_small)()
    state['sd'] = sdb[...].astype(f32).reshape(1, D)
    state['never'] = gm[0:16, 0:128].astype(f32)[0:8, :] > 2.0
    gmax = jnp.max(gm[0:16, 0:128].astype(f32))
    state['z0'] = (gmax > 2.0).astype(jnp.int32)
    state['z1'] = (gmax > 3.0).astype(jnp.int32)
    def front_block(b):
        W(c_in[b])()
        FK(2 * b)(); FK(2 * b + 1)()
        drain(lambda: KVgen(2 * b))(); SD(2 * b)()
        drain(lambda: KVgen(2 * b + 1))(); SD(2 * b + 1)()
        drain(lambda: CVgen(b))()
        INV(2 * b)(); INV(2 * b + 1)()

    def modulation():
        if OPT.get('gpre', 1):
            GPRE(0); GPRE(1)
        for i in range(ND):
            W(c_wmod[i])()
            MOD(i)()
        MODfin()
        mark('modfin')
        drain(lambda: GATEgen(0))(); drain(lambda: GATEgen(1))()
    front_block(0)
    if ORDER1:
        modulation()
        front_block(1)
        drain(lambda: GATEgen(2))(); drain(lambda: GATEgen(3))()
    else:
        front_block(1)
        modulation()

    for s in range(NB):
        h2 = lambda: pltpu.bitcast(h2b[s * RB // 2:(s + 1) * RB // 2, :], bf16)
        for j in range(NF):
            for fn in pre.get((s, 2 * j), []):
                fn()
            g = dot(h2(), tie(wg, D, j * FB, FB, T(s, 2 * j), T(s, 2 * j + 1)))
            for fn in pre.get((s, 2 * j + 1), []):
                fn()
            u = dot(h2(), tie(wu, D, j * FB, FB, T(s, 2 * j + 1), T(s, 2 * j + 2)))
            actb[:, j * FB:(j + 1) * FB] = pltpu.bitcast((jnp.maximum(g, 0.0) * u).astype(bf16), I32)
        for n in range(ND):
            for fn in pre.get((s, 6 + n), []):
                fn()
            p = dot(pltpu.bitcast(actb[...], bf16), tie(wd, FF, n * 128, 128, T(s, 6 + n), T(s, 7 + n)))
            if s == 0:
                pb[:, n * 128:(n + 1) * 128] = p
                continue
            ob[s * RB:(s + 1) * RB, n * 128:(n + 1) * 128] = (
                x1b[s * RB:(s + 1) * RB, n * 128:(n + 1) * 128]
                + state['gb'][:, n * 128:(n + 1) * 128] * p).astype(bf16)
            if s == NB - 1 and SPLIT_LAST:
                last_copy(n).start()
        for fn in pre.get((s, 11), []):
            fn()
        if s != 0 and not (s == NB - 1 and SPLIT_LAST):
            out_copy(s).start()
        mark('step%d' % s)
    for st in streams:
        assert st['done'] == st['n'], st
    for s in range(NB - 1 if SPLIT_LAST else NB):
        out_copy(s).wait()
    if SPLIT_LAST:
        for n in range(ND):
            last_copy(n).wait()
    mark('end')


def _planC(opt, stream, before, T, k):
    W, INV, CV, GATE, FK, SD, KV, drain = k['W'], k['INV'], k['CV'], k['GATE'], k['FK'], k['SD'], k['KV'], k['drain']
    ncv, c_in, c_wgu, c_wd, c_gb = k['ncv'], k['c_in'], k['c_wgu'], k['c_wd'], k['c_gb']
    inv = {s: opt.get('inv', [5, 6]) for s in range(NB)}
    inv[1] = opt.get('inv1', [7, 8])
    slack = opt.get('slack', 0.5)

    def pair(b, s, d, wait=None):
        if wait is not None:
            before(s, d, W(wait))
        if b in opt.get('kvtie', []):
            t0, t1, t2 = T(s - 1, 9), T(s - 1, 10), T(s - 1, 11)
            fr = (np.arange(40) + 1) / 40
            stream(list(t0 + fr * (t1 - t0)), KV(2 * b))
            stream(list(t1 + fr * (t2 - t1)), KV(2 * b + 1))
            busy.append((t0 - T(0, opt.get('kvslack', 0.3)), t2))
            before(s, d, FK(2 * b), FK(2 * b + 1), SD(2 * b), SD(2 * b + 1))
        else:
            before(s, d, FK(2 * b), FK(2 * b + 1), drain(KV(2 * b)), SD(2 * b), drain(KV(2 * b + 1)), SD(2 * b + 1))
        rel[b] = T(s, d)
    busy = []
    rel = {}
    for i, grp in enumerate(c_wgu):
        before(0, i * (6 // len(c_wgu)), W(grp))
    if not opt.get('order1'):
        before(0, opt.get('g23', 2), W(k['c_x1']), drain(GATE(2)), drain(GATE(3)))
    for grp, (n0, n1) in zip(c_wd, opt.get('wdg', [[0, 2], [2, 5]])):
        before(0, 6 + n0, W(grp))
    pos = opt.get('pairs', [[2, 1, 3], [3, 1, 9], [4, 2, 1], [5, 2, 8], [6, 3, 8], [7, 4, 8]])
    for b, s, d in pos:
        fin0 = opt.get('fin0')
        wait = c_in[b] + (c_gb if b == 2 and not fin0 else []) if b <= 4 else None
        pair(b, s, d, wait)
        if b == 2:
            if fin0:
                before(fin0[0], fin0[1], W(c_gb), k['FIN0'])
            else:
                before(s, d, k['FIN0'])
    for s in range(1, NB - 1):
        b = s + 1
        before(s, inv[s][0], INV(2 * b), drain(GATE(2 * b)))
        before(s, inv[s][1], INV(2 * b + 1), drain(GATE(2 * b + 1)))

    if opt.get('fin0late'):
        before(opt['fin0late'][0], opt['fin0late'][1], k['FIN0b'])
    for s, d in opt.get('bars', []):
        before(s, d, k['BAR'])
    _, s_rel, d_rel = pos[0]
    grid = np.arange(T(s_rel, d_rel), T(NB - 2, inv[NB - 2][0] - slack), 8.0)
    ok = np.ones(len(grid), bool)
    for s in range(1, NB - 2):
        ok &= ~((grid >= T(s, inv[s][0] - slack)) & (grid < T(s, inv[s][1] + opt.get('gpause', 2))))
    for b, s, d in pos:
        ok &= ~((grid >= T(s, d)) & (grid < T(s, d + opt.get('ppause', 0.4))))
    for lo, hi in busy:
        ok &= ~((grid >= lo) & (grid < hi))
    grid = grid[ok]
    total = sum(4 * b + 3 for b in range(2, NB))
    a = 0.0
    for b in range(2, NB):
        n = ncv(b)
        dead = np.searchsorted(grid, T(b - 1, inv[b - 1][0] - slack)) - 1
        first = max(a, np.searchsorted(grid, rel[b]))
        last = min(first + (4 * b + 3) / total * len(grid) * opt.get('pace', 1.0), dead)
        idx = first + (np.arange(n) + 1) / n * (last - first)
        stream(list(grid[np.minimum(idx.astype(int), len(grid) - 1)]), CV(b))
        a = last


@jax.jit
def pallas_adaLN_cond__ssm_conv_h3__glu_gated_reglu__prompt_kernel(
        A_q, A_k, A_v, A_shift_k, A_ssm_k, A_ssm_D, B_x, B_W_gate, B_W_up, B_W_down, c, w_mod):
    bf16, f32 = jnp.bfloat16, jnp.float32
    any_spec = pl.BlockSpec(memory_space=pl.ANY)
    V = pltpu.VMEM
    out = pl.pallas_call(
        _kernel,
        out_shape=jax.ShapeDtypeStruct((S, D), bf16),
        in_specs=[any_spec] * 13,
        out_specs=any_spec,
        scratch_shapes=[
            V((1, D), bf16), V((4, D), bf16), V((D,), bf16),
            V((S, D), bf16), V((S, D), bf16), V((S, D), bf16),
            V((D, S), bf16),
            V((D, FF), bf16), V((D, FF), bf16), V((FF, D), bf16),
            V((D, 6 * D), bf16),
            V((2 * L0, L0), bf16), V((L0, 2 * L0), bf16),
            V((S // 2, D), I32),
            V((ND, NC, 2 * L0, 128), f32), V((ND, NC, 2 * L0, 128), f32),
            V((ND, NC, L0, 128), I32),
            V((ND, 2 * L0, 128), f32),
            V((S // 2, D), I32), V((S, D), f32), V((RB // 2, FF), I32), V((8, 6 * D), f32), V((S, D), bf16), V((RB, D), f32),
            pltpu.SemaphoreType.DMA((NSEM,)), pltpu.SemaphoreType.DMA, pltpu.SemaphoreType.REGULAR,
        ],
        compiler_params=pltpu.CompilerParams(vmem_limit_bytes=110 * 1024 * 1024,
                                             disable_semaphore_checks=bool(OPT.get('nosemchk', 0)), flags=OPT.get('flags')),
    )(c, A_shift_k.T, A_ssm_D,
      A_q.reshape(S, D), A_k.reshape(S, D), A_v.reshape(S, D), A_ssm_k,
      B_W_gate, B_W_up, B_W_down, w_mod, jnp.asarray(_FB), jnp.asarray(_GB))
    return out.reshape(1, S, D)
```

```python
import numpy as np
import jax
import jax.numpy as jnp
from jax import lax
import jax.experimental.pallas as pl
import jax.experimental.pallas.tpu as pltpu

S, D, FF = 2048, 640, 1536
L0 = 128
NC = S // L0
ND = D // 128
NT = ND * (L0 // 8)
RB = 256
NB = S // RB
FB = 512
NF = FF // FB
EPS = 1e-5
I32 = jnp.int32

_CUM = np.concatenate([[0], np.cumsum([1280] * 6 + [768] * 5)])

INV_AT = [None, (9, 10)] + [(5, 6)] * (NB - 3)
SPECTRA_AT = {2: (1, 3), 3: (1, 7), 4: (2, 0), 5: (3, 0), 6: (4, 0), 7: (5, 0)}
FENCES = [(2, 0), (3, 0), (4, 0), (5, 0), (6, 0)]
WD_GROUPS = [(0, 2), (2, 5)]
INV_SLACK, GATE_PAUSE, SPECTRA_PAUSE, RELEASE_PAUSE = 0.5, 2.5, 0.4, 2.0


def _dft_mats():
    n = np.arange(L0, dtype=np.float64)
    w = np.pi * (4 * n + 1) / (2 * L0)
    ang = w[:, None] * n[None, :]
    fr, fi = np.cos(ang), -np.sin(ang)
    F = np.stack([fr.reshape(L0 // 8, 8, L0), fi.reshape(L0 // 8, 8, L0)], axis=1).reshape(2 * L0, L0)
    G = np.stack([fr.T.reshape(L0, L0 // 8, 8), fi.T.reshape(L0, L0 // 8, 8)], axis=-1).reshape(L0, 2 * L0) / L0
    return F.astype(np.float32).astype(jnp.bfloat16), G.astype(np.float32).astype(jnp.bfloat16)


_FB, _GB = _dft_mats()


def _time(s, d):
    return s * float(_CUM[-1]) + float(np.interp(d, np.arange(12), _CUM))


def _phases(b):
    return 2 if b >= 2 else 1


def _conv_deadlines():
    grid = np.arange(_time(*SPECTRA_AT[2]), _time(NB - 2, INV_AT[NB - 2][0] - INV_SLACK), 8.0)
    ok = np.ones(len(grid), bool)
    for s in range(1, NB - 2):
        ok &= ~((grid >= _time(s, INV_AT[s][0] - INV_SLACK)) & (grid < _time(s, INV_AT[s][1] + GATE_PAUSE)))
    for s, d in SPECTRA_AT.values():
        ok &= ~((grid >= _time(s, d)) & (grid < _time(s, d + SPECTRA_PAUSE)))
    grid = grid[ok]
    total = sum(4 * b + 3 for b in range(2, NB))
    out, a = {}, 0.0
    for b in range(2, NB):
        n = NT * _phases(b)
        dead = np.searchsorted(grid, _time(b - 1, INV_AT[b - 1][0] - INV_SLACK)) - 1
        first = max(a, np.searchsorted(grid, _time(*SPECTRA_AT[b]) + _time(0, RELEASE_PAUSE)))
        a = min(first + (4 * b + 3) / total * len(grid), dead)
        idx = first + (np.arange(n) + 1) / n * (a - first)
        out[b] = list(grid[np.minimum(idx.astype(int), len(grid) - 1)])
    return out


def _ln(x):
    m = jnp.mean(x, axis=-1, keepdims=True)
    xc = x - m
    v = jnp.mean(xc * xc, axis=-1, keepdims=True)
    return xc * lax.rsqrt(v + EPS)


def _dot(a, b):
    return jnp.dot(a, b, preferred_element_type=jnp.float32)


def _kernel(c_hbm, sk_hbm, sd_hbm, x_hbm, k_hbm, v_hbm, ssmk_hbm, wg_hbm, wu_hbm, wd_hbm,
            wmod_hbm, f_hbm, g_hbm, o_hbm,
            cb, skb, sdb, xb, kb, vb, ssmk, wg, wu, wd, wmod, fm, gm,
            kvb, uf, kf, wf, zs, h2b, x1b, actb, ob, pb, sems, osem, fsem):
    f32, bf16 = jnp.float32, jnp.bfloat16

    nsem = [0]

    def group(pairs):
        sem = sems.at[nsem[0]]
        nsem[0] += 1
        return [pltpu.make_async_copy(src, dst, sem) for src, dst in pairs]

    def rows(src, dst, lo, n):
        return src.at[pl.ds(lo, n), :], dst.at[pl.ds(lo, n), :]

    def cols(src, dst, lo, n):
        return src.at[:, pl.ds(lo, n)], dst.at[:, pl.ds(lo, n)]

    def inputs(blocks, with_x=True):
        return group([p for b in blocks for p in (
            [cols(ssmk_hbm, ssmk, b * RB, RB), rows(k_hbm, kb, b * RB, RB), rows(v_hbm, vb, b * RB, RB)]
            + ([rows(x_hbm, xb, b * RB, RB)] if with_x else []))])

    def wait(*groups):
        for grp in groups:
            for cpy in grp:
                cpy.wait()

    c_small = group([(f_hbm, fm), (c_hbm, cb), (sk_hbm, skb), (sd_hbm, sdb), (g_hbm, gm)])
    c_in = {0: inputs([0]), 2: inputs([2]), 3: inputs([3]), 4: inputs([4, 5, 6, 7]), 1: inputs([1], False)}
    c_x1 = group([rows(x_hbm, xb, RB, RB)])
    c_wmod = [group([(wmod_hbm.at[pl.ds(i * 128, 128), pl.ds(0, 5 * D)], wmod.at[pl.ds(i * 128, 128), pl.ds(0, 5 * D)])])
              for i in range(ND)]
    c_gb = group([cols(wmod_hbm, wmod, 5 * D, D)])
    c_wgu = [group([cols(src, dst, j * FB, FB)]) for j in range(NF) for src, dst in ((wg_hbm, wg), (wu_hbm, wu))]
    c_wd = [group([cols(wd_hbm, wd, n * 128, 128) for n in range(n0, n1)]) for n0, n1 in WD_GROUPS]
    assert nsem[0] == sems.shape[0]
    for grp in ([c_small, c_in[0], c_in[1]] + c_wmod + c_wgu[:2] + [c_x1] + c_wgu[2:] + c_wd
                + [c_in[2], c_gb, c_in[3], c_in[4]]):
        for cpy in grp:
            cpy.start()

    def out_copy(s):
        return pltpu.make_async_copy(*rows(ob, o_hbm, s * RB, RB), osem)

    def last_copy(n):
        r, c = pl.ds((NB - 1) * RB, RB), pl.ds(n * 128, 128)
        return pltpu.make_async_copy(ob.at[r, c], o_hbm.at[r, c], osem)

    def filter_spectrum(c):
        r = lax.dot_general(fm[...], ssmk[:, c * L0:(c + 1) * L0], (((1,), (1,)), ((), ())),
                            preferred_element_type=f32)
        for dt in range(ND):
            kf[dt, c] = r[:, dt * 128:(dt + 1) * 128]

    def signal_spectrum(j):
        sk = skb[...].astype(f32)
        r0 = j * L0
        kc = kb[r0:r0 + L0, :].astype(f32)
        prev = jnp.zeros((8, D), f32) if j == 0 else kb[r0 - 16:r0, :].astype(f32)[8:, :]
        ext = jnp.concatenate([prev, kc], axis=0)
        acc = kc * sk[0:1, :]
        for t in range(1, 4):
            acc = acc + pltpu.roll(ext, t, axis=0)[8:, :] * sk[t:t + 1, :]
        kvb[r0 // 2:(r0 + L0) // 2, :] = pltpu.bitcast((acc * vb[r0:r0 + L0, :].astype(f32)).astype(bf16), I32)
        r = _dot(fm[...], pltpu.bitcast(kvb[r0 // 2:(r0 + L0) // 2, :], bf16))
        for dt in range(ND):
            uf[dt, j] = r[:, dt * 128:(dt + 1) * 128]

    def spectra(b):
        filter_spectrum(2 * b)
        filter_spectrum(2 * b + 1)
        signal_spectrum(2 * b)
        signal_spectrum(2 * b + 1)

    def conv_tile(b, t):
        dt, ft = t // 16, t % 16
        re, im = slice(ft * 16, ft * 16 + 8), slice(ft * 16 + 8, ft * 16 + 16)
        a0, a1 = 2 * b, 2 * b + 1

        def mac(z, kr, ki, ur, ui):
            pr, pi = kr * ur - ki * ui, kr * ui + ki * ur
            return (pr, pi) if z is None else (z[0] + pr, z[1] + pi)
        z0 = z1 = None
        u = (uf[dt, a1, re, :], uf[dt, a1, im, :])
        mid = (a1 + 1) // 2 - 1 if _phases(b) == 2 else -1
        for c in range(a1 + 1):
            kr, ki = kf[dt, c, re, :], kf[dt, c, im, :]
            z1 = mac(z1, kr, ki, *u)
            if c <= a0:
                u = (uf[dt, a0 - c, re, :], uf[dt, a0 - c, im, :])
                z0 = mac(z0, kr, ki, *u)
            if c == mid:
                yield pltpu.bitcast(z1[0] + z1[1] + z0[0] + z0[1], I32)
        w0r, w0i = z0 if b == 0 else (z0[0] - zs[dt, im, :], z0[1] + zs[dt, re, :])
        w1r, w1i = z1[0] - z0[1], z1[1] + z0[0]
        if b < NB - 1:
            zs[dt, re, :] = z1[0]
            zs[dt, im, :] = z1[1]
        w0 = pltpu.pack_elementwise([w0r, w0i], packed_dtype=bf16)
        w1 = pltpu.pack_elementwise([w1r, w1i], packed_dtype=bf16)
        wf[dt, a0, ft * 8:ft * 8 + 8, :] = w0
        wf[dt, a1, ft * 8:ft * 8 + 8, :] = w1
        yield w0 | w1

    def conv(b):
        for t in range(NT):
            yield from conv_tile(b, t)

    def inverse(a):
        return _dot(gm[...], jnp.concatenate([pltpu.bitcast(wf[dt, a], bf16) for dt in range(ND)], axis=1))

    mod = {}

    def gate_pre(a, y):
        r0 = a * L0
        x = xb[r0:r0 + L0, :].astype(f32)
        kvd = pltpu.bitcast(kvb[r0 // 2:(r0 + L0) // 2, :], bf16).astype(f32) * mod['sd']
        return x, _ln(x), y + kvd

    def gate(a, pre):
        r0 = a * L0
        x, xn, t = pre
        x1 = x + mod['ga'] * ((xn * mod['ca1'] + mod['sa']) * t)
        x1b[r0:r0 + L0, :] = x1
        h2 = (_ln(x1) * mod['cb1'] + mod['sb']).astype(bf16)
        h2b[r0 // 2:(r0 + L0) // 2, :] = pltpu.bitcast(h2, I32)

    def finish(s, n, p):
        r, c = slice(s * RB, (s + 1) * RB), slice(n * 128, (n + 1) * 128)
        ob[r, c] = (x1b[r, c] + mod['gb'][:, c] * p).astype(bf16)

    wait(c_small)
    mod['sd'] = sdb[...].astype(f32).reshape(1, D)
    never = gm[0:16, 0:128].astype(f32)[0:8, :] > 2.0
    ys = {}
    for b in range(2):
        wait(c_in[b])
        spectra(b)
        for _ in conv(b):
            pass
        ys[2 * b], ys[2 * b + 1] = inverse(2 * b), inverse(2 * b + 1)
    pres = [gate_pre(0, ys[0]), gate_pre(1, ys[1])]
    for i in range(ND):
        wait(c_wmod[i])
        if i == 0:
            cc = cb[...].astype(f32)
            mod['sc'] = jnp.broadcast_to((cc * jax.nn.sigmoid(cc)).astype(bf16), (16, D))
        p = _dot(mod['sc'][:, i * 128:(i + 1) * 128], wmod[i * 128:(i + 1) * 128, 0:5 * D])[0:8, :]
        m = p if i == 0 else m + p
    m = m[0:1, :]
    mod.update(sa=m[:, 0:D], ca1=1.0 + m[:, D:2 * D], ga=m[:, 2 * D:3 * D], sb=m[:, 3 * D:4 * D],
               cb1=1.0 + m[:, 4 * D:5 * D])
    gate(0, pres[0])
    gate(1, pres[1])

    due = _conv_deadlines()
    tiles = {b: [conv(b), 0] for b in due}
    wregs = {}

    def next_tile(t):
        for b, st in tiles.items():
            if st[1] < len(due[b]) and due[b][st[1]] <= t + 1e-6:
                if all(o[1] >= len(due[ob_]) or due[ob_][o[1]] >= due[b][st[1]] for ob_, o in tiles.items()):
                    st[1] += 1
                    return next(st[0])
        return None

    def weights(wref, nr, c0, nc, s, d):
        nk, nn = nr // 128, nc // 128
        t0, t1 = _time(s, d), _time(s, d + 1)
        blocks, i = {}, 0
        for nt in range(nn):
            for kt in range(nk):
                pcs = []
                for r in range(8):
                    i += 1
                    key = (id(wref), kt * 128 + r * 16, c0 + nt * 128)
                    if key not in wregs:
                        wregs[key] = wref[key[1]:key[1] + 16, key[2]:key[2] + 128]
                    w = wregs[key]
                    tok = next_tile(t0 + (t1 - t0) * i / (nk * nn * 8))
                    if tok is not None:
                        w = pltpu.bitcast(jnp.where(never, tok, pltpu.bitcast(w, I32)), bf16)
                    pcs.append(w)
                blocks[kt, nt] = jnp.concatenate(pcs, axis=0)
        return jnp.concatenate([jnp.concatenate([blocks[kt, nt] for nt in range(nn)], axis=1)
                                for kt in range(nk)], axis=0)

    def between(s, d):
        if s == 0:
            if d < 6:
                wait(c_wgu[d])
            if d == 4:
                wait(c_x1)
                gate(2, gate_pre(2, ys[2]))
                gate(3, gate_pre(3, ys[3]))
            for grp, (n0, _) in zip(c_wd, WD_GROUPS):
                if d == 6 + n0:
                    wait(grp)
        for b, at in SPECTRA_AT.items():
            if at == (s, d):
                if b <= 4:
                    wait(c_in[b])
                if b == 2:
                    wait(c_gb)
                spectra(b)
                if b == 2:
                    mod['gb'] = _dot(mod['sc'], wmod[:, 5 * D:6 * D])[0:1, :]
        if 1 <= s < NB - 1 and d in INV_AT[s]:
            a = 2 * s + 2 + INV_AT[s].index(d)
            assert tiles[s + 1][1] == len(due[s + 1])
            gate(a, gate_pre(a, inverse(a)))
        if (s, d) == (NB - 1, 1):
            for n in range(ND):
                finish(0, n, pb[:, n * 128:(n + 1) * 128])
            out_copy(0).start()
        if (s, d) in FENCES:
            pl.semaphore_signal(fsem, 1)
            pl.semaphore_wait(fsem, 1)

    for s in range(NB):
        for j in range(NF):
            between(s, 2 * j)
            g = _dot(pltpu.bitcast(h2b[s * RB // 2:(s + 1) * RB // 2, :], bf16), weights(wg, D, j * FB, FB, s, 2 * j))
            between(s, 2 * j + 1)
            u = _dot(pltpu.bitcast(h2b[s * RB // 2:(s + 1) * RB // 2, :], bf16), weights(wu, D, j * FB, FB, s, 2 * j + 1))
            actb[:, j * FB:(j + 1) * FB] = pltpu.bitcast((jnp.maximum(g, 0.0) * u).astype(bf16), I32)
        for n in range(ND):
            between(s, 6 + n)
            p = _dot(pltpu.bitcast(actb[...], bf16), weights(wd, FF, n * 128, 128, s, 6 + n))
            if s == 0:
                pb[:, n * 128:(n + 1) * 128] = p
            else:
                finish(s, n, p)
            if s == NB - 1:
                last_copy(n).start()
        if 0 < s < NB - 1:
            out_copy(s).start()
    assert all(st[1] == len(due[b]) for b, st in tiles.items())
    for s in range(NB - 1):
        out_copy(s).wait()
    for n in range(ND):
        last_copy(n).wait()


@jax.jit
def pallas_adaLN_cond__ssm_conv_h3__glu_gated_reglu__prompt_kernel(
        A_q, A_k, A_v, A_shift_k, A_ssm_k, A_ssm_D, B_x, B_W_gate, B_W_up, B_W_down, c, w_mod):
    del B_x
    bf16, f32 = jnp.bfloat16, jnp.float32
    hbm = pl.BlockSpec(memory_space=pl.ANY)
    V = pltpu.VMEM
    out = pl.pallas_call(
        _kernel,
        out_shape=jax.ShapeDtypeStruct((S, D), bf16),
        in_specs=[hbm] * 13,
        out_specs=hbm,
        scratch_shapes=[
            V((1, D), bf16), V((4, D), bf16), V((D,), bf16),
            V((S, D), bf16), V((S, D), bf16), V((S, D), bf16),
            V((D, S), bf16),
            V((D, FF), bf16), V((D, FF), bf16), V((FF, D), bf16),
            V((D, 6 * D), bf16),
            V((2 * L0, L0), bf16), V((L0, 2 * L0), bf16),
            V((S // 2, D), I32),
            V((ND, NC, 2 * L0, 128), f32), V((ND, NC, 2 * L0, 128), f32),
            V((ND, NC, L0, 128), I32),
            V((ND, 2 * L0, 128), f32),
            V((S // 2, D), I32), V((S, D), f32),
            V((RB // 2, FF), I32), V((S, D), bf16), V((RB, D), f32),
            pltpu.SemaphoreType.DMA((21,)), pltpu.SemaphoreType.DMA, pltpu.SemaphoreType.REGULAR,
        ],
        compiler_params=pltpu.CompilerParams(vmem_limit_bytes=110 * 1024 * 1024),
    )(c, A_shift_k.T, A_ssm_D,
      A_q.reshape(S, D), A_k.reshape(S, D), A_v.reshape(S, D), A_ssm_k,
      B_W_gate, B_W_up, B_W_down, w_mod, jnp.asarray(_FB), jnp.asarray(_GB))
    return out.reshape(1, S, D)
```

```python
import numpy as np
import jax
import jax.numpy as jnp
from jax import lax
import jax.experimental.pallas as pl
import jax.experimental.pallas.tpu as pltpu

S, D, FF = 2048, 640, 1536
L0 = 128
NC = S // L0
ND = D // 128
NT = ND * (L0 // 8)
RB = 256
NB = S // RB
FB = 512
NF = FF // FB
EPS = 1e-5
I32 = jnp.int32

_CUM = np.concatenate([[0], np.cumsum([1280] * 6 + [768] * 5)])

INV_AT = [None, (9, 10)] + [(5, 6)] * (NB - 3)
SPECTRA_AT = {2: (1, 3), 3: (1, 7), 4: (2, 0), 5: (3, 0), 6: (4, 0), 7: (5, 0)}
FENCES = [(2, 0), (3, 0), (4, 0), (5, 0), (6, 0)]
WD_GROUPS = [(0, 2), (2, 5)]
INV_SLACK, GATE_PAUSE, SPECTRA_PAUSE, RELEASE_PAUSE = 0.5, 2.5, 0.4, 2.5


def _dft_mats():
    n = np.arange(L0, dtype=np.float64)
    w = np.pi * (4 * n + 1) / (2 * L0)
    ang = w[:, None] * n[None, :]
    fr, fi = np.cos(ang), -np.sin(ang)
    F = np.stack([fr.reshape(L0 // 8, 8, L0), fi.reshape(L0 // 8, 8, L0)], axis=1).reshape(2 * L0, L0)
    G = F.T / L0
    return F.astype(np.float32).astype(jnp.bfloat16), G.astype(np.float32).astype(jnp.bfloat16)


_FB, _GB = _dft_mats()


def _time(s, d):
    return s * float(_CUM[-1]) + float(np.interp(d, np.arange(12), _CUM))


def _phases(b):
    return 2 if b >= 2 else 1


def _conv_deadlines():
    grid = np.arange(_time(*SPECTRA_AT[2]), _time(NB - 2, INV_AT[NB - 2][0] - INV_SLACK), 8.0)
    ok = np.ones(len(grid), bool)
    for s in range(1, NB - 2):
        ok &= ~((grid >= _time(s, INV_AT[s][0] - INV_SLACK)) & (grid < _time(s, INV_AT[s][1] + GATE_PAUSE)))
    for s, d in SPECTRA_AT.values():
        ok &= ~((grid >= _time(s, d)) & (grid < _time(s, d + SPECTRA_PAUSE)))
    grid = grid[ok]
    total = sum(4 * b + 3 for b in range(2, NB))
    out, a = {}, 0.0
    for b in range(2, NB):
        n = NT * _phases(b)
        dead = np.searchsorted(grid, _time(b - 1, INV_AT[b - 1][0] - INV_SLACK)) - 1
        first = max(a, np.searchsorted(grid, _time(*SPECTRA_AT[b]) + _time(0, RELEASE_PAUSE)))
        a = min(first + (4 * b + 3) / total * len(grid), dead)
        idx = first + (np.arange(n) + 1) / n * (a - first)
        out[b] = list(grid[np.minimum(idx.astype(int), len(grid) - 1)])
    return out


def _ln(x):
    m = jnp.mean(x, axis=-1, keepdims=True)
    xc = x - m
    v = jnp.mean(xc * xc, axis=-1, keepdims=True)
    return xc * lax.rsqrt(v + EPS)


def _dot(a, b):
    return jnp.dot(a, b, preferred_element_type=jnp.float32)


def _kernel(c_hbm, sk_hbm, sd_hbm, x_hbm, k_hbm, v_hbm, ssmk_hbm, wg_hbm, wu_hbm, wd_hbm,
            wmod_hbm, f_hbm, g_hbm, o_hbm,
            cb, skb, sdb, xb, kb, vb, ssmk, wg, wu, wd, wmod, fm, gm,
            kvb, uf, kf, wf, zs, h2b, x1b, actb, ob, pb, sems, osem, fsem):
    f32, bf16 = jnp.float32, jnp.bfloat16

    nsem = [0]

    def group(pairs):
        sem = sems.at[nsem[0]]
        nsem[0] += 1
        return [pltpu.make_async_copy(src, dst, sem) for src, dst in pairs]

    def rows(src, dst, lo, n):
        return src.at[pl.ds(lo, n), :], dst.at[pl.ds(lo, n), :]

    def cols(src, dst, lo, n):
        return src.at[:, pl.ds(lo, n)], dst.at[:, pl.ds(lo, n)]

    def inputs(blocks, with_x=True):
        return group([p for b in blocks for p in (
            [cols(ssmk_hbm, ssmk, b * RB, RB), rows(k_hbm, kb, b * RB, RB), rows(v_hbm, vb, b * RB, RB)]
            + ([rows(x_hbm, xb, b * RB, RB)] if with_x else []))])

    def wait(*groups):
        for grp in groups:
            for cpy in grp:
                cpy.wait()

    c_small = group([(f_hbm, fm), (c_hbm, cb), (sk_hbm, skb), (sd_hbm, sdb), (g_hbm, gm)])
    c_in = {0: inputs([0]), 2: inputs([2]), 3: inputs([3]), 4: inputs([4, 5, 6, 7]), 1: inputs([1], False)}
    c_x1 = group([rows(x_hbm, xb, RB, RB)])
    c_wmod = [group([(wmod_hbm.at[pl.ds(i * 128, 128), pl.ds(0, 5 * D)], wmod.at[pl.ds(i * 128, 128), pl.ds(0, 5 * D)])])
              for i in range(ND)]
    c_gb = group([cols(wmod_hbm, wmod, 5 * D, D)])
    c_wgu = [group([cols(src, dst, j * FB, FB)]) for j in range(NF) for src, dst in ((wg_hbm, wg), (wu_hbm, wu))]
    c_wd = [group([cols(wd_hbm, wd, n * 128, 128) for n in range(n0, n1)]) for n0, n1 in WD_GROUPS]
    assert nsem[0] == sems.shape[0]
    for grp in ([c_small, c_in[0], c_in[1]] + c_wmod + c_wgu[:2] + [c_x1] + c_wgu[2:] + c_wd
                + [c_in[2], c_gb, c_in[3], c_in[4]]):
        for cpy in grp:
            cpy.start()

    def out_copy(s):
        return pltpu.make_async_copy(*rows(ob, o_hbm, s * RB, RB), osem)

    def last_copy(n):
        r, c = pl.ds((NB - 1) * RB, RB), pl.ds(n * 128, 128)
        return pltpu.make_async_copy(ob.at[r, c], o_hbm.at[r, c], osem)

    def filter_spectrum(c):
        r = lax.dot_general(fm[...], ssmk[:, c * L0:(c + 1) * L0], (((1,), (1,)), ((), ())),
                            preferred_element_type=f32)
        for dt in range(ND):
            kf[dt, c] = r[:, dt * 128:(dt + 1) * 128]

    def signal_spectrum(j):
        sk = skb[...].astype(f32)
        r0 = j * L0
        kc = kb[r0:r0 + L0, :].astype(f32)
        prev = jnp.zeros((8, D), f32) if j == 0 else kb[r0 - 16:r0, :].astype(f32)[8:, :]
        ext = jnp.concatenate([prev, kc], axis=0)
        acc = kc * sk[0:1, :]
        for t in range(1, 4):
            acc = acc + pltpu.roll(ext, t, axis=0)[8:, :] * sk[t:t + 1, :]
        kvb[r0 // 2:(r0 + L0) // 2, :] = pltpu.bitcast((acc * vb[r0:r0 + L0, :].astype(f32)).astype(bf16), I32)
        r = _dot(fm[...], pltpu.bitcast(kvb[r0 // 2:(r0 + L0) // 2, :], bf16))
        for dt in range(ND):
            uf[dt, j] = r[:, dt * 128:(dt + 1) * 128]

    def spectra(b):
        filter_spectrum(2 * b)
        filter_spectrum(2 * b + 1)
        signal_spectrum(2 * b)
        signal_spectrum(2 * b + 1)

    def conv_tile(b, t):
        dt, ft = t // 16, t % 16
        re, im = slice(ft * 16, ft * 16 + 8), slice(ft * 16 + 8, ft * 16 + 16)
        a0, a1 = 2 * b, 2 * b + 1

        def mac(z, kr, ki, ur, ui):
            pr, pi = kr * ur - ki * ui, kr * ui + ki * ur
            return (pr, pi) if z is None else (z[0] + pr, z[1] + pi)
        z0 = z1 = None
        u = (uf[dt, a1, re, :], uf[dt, a1, im, :])
        mid = (a1 + 1) // 2 - 1 if _phases(b) == 2 else -1
        for c in range(a1 + 1):
            kr, ki = kf[dt, c, re, :], kf[dt, c, im, :]
            z1 = mac(z1, kr, ki, *u)
            if c <= a0:
                u = (uf[dt, a0 - c, re, :], uf[dt, a0 - c, im, :])
                z0 = mac(z0, kr, ki, *u)
            if c == mid:
                yield pltpu.bitcast(z1[0] + z1[1] + z0[0] + z0[1], I32)
        w0r, w0i = z0 if b == 0 else (z0[0] - zs[dt, im, :], z0[1] + zs[dt, re, :])
        w1r, w1i = z1[0] - z0[1], z1[1] + z0[0]
        if b < NB - 1:
            zs[dt, re, :] = z1[0]
            zs[dt, im, :] = z1[1]
        w0 = pltpu.bitcast(jnp.concatenate([w0r, w0i], axis=0).astype(bf16), I32)
        w1 = pltpu.bitcast(jnp.concatenate([w1r, w1i], axis=0).astype(bf16), I32)
        wf[dt, a0, ft * 8:ft * 8 + 8, :] = w0
        wf[dt, a1, ft * 8:ft * 8 + 8, :] = w1
        yield w0 | w1

    def conv(b):
        for t in range(NT):
            yield from conv_tile(b, t)

    def inverse(a):
        return _dot(gm[...], jnp.concatenate([pltpu.bitcast(wf[dt, a], bf16) for dt in range(ND)], axis=1))

    mod = {}

    def gate_pre(a, y):
        r0 = a * L0
        x = xb[r0:r0 + L0, :].astype(f32)
        kvd = pltpu.bitcast(kvb[r0 // 2:(r0 + L0) // 2, :], bf16).astype(f32) * mod['sd']
        return x, _ln(x), y + kvd

    def gate(a, pre):
        r0 = a * L0
        x, xn, t = pre
        x1 = x + mod['ga'] * ((xn * mod['ca1'] + mod['sa']) * t)
        x1b[r0:r0 + L0, :] = x1
        h2 = (_ln(x1) * mod['cb1'] + mod['sb']).astype(bf16)
        h2b[r0 // 2:(r0 + L0) // 2, :] = pltpu.bitcast(h2, I32)

    def finish(s, n, p):
        r, c = slice(s * RB, (s + 1) * RB), slice(n * 128, (n + 1) * 128)
        ob[r, c] = (x1b[r, c] + mod['gb'][:, c] * p).astype(bf16)

    wait(c_small)
    mod['sd'] = sdb[...].astype(f32).reshape(1, D)
    never = gm[0:16, 0:128].astype(f32)[0:8, :] > 2.0
    ys = {}
    for b in range(2):
        wait(c_in[b])
        spectra(b)
        for _ in conv(b):
            pass
        ys[2 * b], ys[2 * b + 1] = inverse(2 * b), inverse(2 * b + 1)
    pres = [gate_pre(0, ys[0]), gate_pre(1, ys[1])]
    for i in range(ND):
        wait(c_wmod[i])
        if i == 0:
            cc = cb[...].astype(f32)
            mod['sc'] = jnp.broadcast_to((cc * jax.nn.sigmoid(cc)).astype(bf16), (16, D))
        p = _dot(mod['sc'][:, i * 128:(i + 1) * 128], wmod[i * 128:(i + 1) * 128, 0:5 * D])[0:8, :]
        m = p if i == 0 else m + p
    m = m[0:1, :]
    mod.update(sa=m[:, 0:D], ca1=1.0 + m[:, D:2 * D], ga=m[:, 2 * D:3 * D], sb=m[:, 3 * D:4 * D],
               cb1=1.0 + m[:, 4 * D:5 * D])
    gate(0, pres[0])
    gate(1, pres[1])

    due = _conv_deadlines()
    tiles = {b: [conv(b), 0] for b in due}
    wregs = {}

    def next_tile(t):
        for b, st in tiles.items():
            if st[1] < len(due[b]) and due[b][st[1]] <= t + 1e-6:
                if all(o[1] >= len(due[ob_]) or due[ob_][o[1]] >= due[b][st[1]] for ob_, o in tiles.items()):
                    st[1] += 1
                    return next(st[0])
        return None

    def weights(wref, nr, c0, nc, s, d):
        nk, nn = nr // 128, nc // 128
        t0, t1 = _time(s, d), _time(s, d + 1)
        blocks, i = {}, 0
        for nt in range(nn):
            for kt in range(nk):
                pcs = []
                for r in range(8):
                    i += 1
                    key = (id(wref), kt * 128 + r * 16, c0 + nt * 128)
                    if key not in wregs:
                        wregs[key] = wref[key[1]:key[1] + 16, key[2]:key[2] + 128]
                    w = wregs[key]
                    tok = next_tile(t0 + (t1 - t0) * i / (nk * nn * 8))
                    if tok is not None:
                        w = pltpu.bitcast(jnp.where(never, tok, pltpu.bitcast(w, I32)), bf16)
                    pcs.append(w)
                blocks[kt, nt] = jnp.concatenate(pcs, axis=0)
        return jnp.concatenate([jnp.concatenate([blocks[kt, nt] for nt in range(nn)], axis=1)
                                for kt in range(nk)], axis=0)

    def between(s, d):
        if s == 0:
            if d < 6:
                wait(c_wgu[d])
            if d == 4:
                wait(c_x1)
                gate(2, gate_pre(2, ys[2]))
                gate(3, gate_pre(3, ys[3]))
            for grp, (n0, _) in zip(c_wd, WD_GROUPS):
                if d == 6 + n0:
                    wait(grp)
        for b, at in SPECTRA_AT.items():
            if at == (s, d):
                if b <= 4:
                    wait(c_in[b])
                if b == 2:
                    wait(c_gb)
                spectra(b)
                if b == 2:
                    mod['gb'] = _dot(mod['sc'], wmod[:, 5 * D:6 * D])[0:1, :]
        if 1 <= s < NB - 1 and d in INV_AT[s]:
            a = 2 * s + 2 + INV_AT[s].index(d)
            assert tiles[s + 1][1] == len(due[s + 1])
            gate(a, gate_pre(a, inverse(a)))
        if (s, d) == (NB - 1, 1):
            for n in range(ND):
                finish(0, n, pb[:, n * 128:(n + 1) * 128])
            out_copy(0).start()
        if (s, d) in FENCES:
            pl.semaphore_signal(fsem, 1)
            pl.semaphore_wait(fsem, 1)

    for s in range(NB):
        for j in range(NF):
            between(s, 2 * j)
            g = _dot(pltpu.bitcast(h2b[s * RB // 2:(s + 1) * RB // 2, :], bf16), weights(wg, D, j * FB, FB, s, 2 * j))
            between(s, 2 * j + 1)
            u = _dot(pltpu.bitcast(h2b[s * RB // 2:(s + 1) * RB // 2, :], bf16), weights(wu, D, j * FB, FB, s, 2 * j + 1))
            actb[:, j * FB:(j + 1) * FB] = pltpu.bitcast((jnp.maximum(g, 0.0) * u).astype(bf16), I32)
        for n in range(ND):
            between(s, 6 + n)
            p = _dot(pltpu.bitcast(actb[...], bf16), weights(wd, FF, n * 128, 128, s, 6 + n))
            if s == 0:
                pb[:, n * 128:(n + 1) * 128] = p
            else:
                finish(s, n, p)
            if s == NB - 1:
                last_copy(n).start()
        if 0 < s < NB - 1:
            out_copy(s).start()
    assert all(st[1] == len(due[b]) for b, st in tiles.items())
    for s in range(NB - 1):
        out_copy(s).wait()
    for n in range(ND):
        last_copy(n).wait()


@jax.jit
def pallas_adaLN_cond__ssm_conv_h3__glu_gated_reglu__prompt_kernel(
        A_q, A_k, A_v, A_shift_k, A_ssm_k, A_ssm_D, B_x, B_W_gate, B_W_up, B_W_down, c, w_mod):
    del B_x
    bf16, f32 = jnp.bfloat16, jnp.float32
    hbm = pl.BlockSpec(memory_space=pl.ANY)
    V = pltpu.VMEM
    out = pl.pallas_call(
        _kernel,
        out_shape=jax.ShapeDtypeStruct((S, D), bf16),
        in_specs=[hbm] * 13,
        out_specs=hbm,
        scratch_shapes=[
            V((1, D), bf16), V((4, D), bf16), V((D,), bf16),
            V((S, D), bf16), V((S, D), bf16), V((S, D), bf16),
            V((D, S), bf16),
            V((D, FF), bf16), V((D, FF), bf16), V((FF, D), bf16),
            V((D, 6 * D), bf16),
            V((2 * L0, L0), bf16), V((L0, 2 * L0), bf16),
            V((S // 2, D), I32),
            V((ND, NC, 2 * L0, 128), f32), V((ND, NC, 2 * L0, 128), f32),
            V((ND, NC, L0, 128), I32),
            V((ND, 2 * L0, 128), f32),
            V((S // 2, D), I32), V((S, D), f32),
            V((RB // 2, FF), I32), V((S, D), bf16), V((RB, D), f32),
            pltpu.SemaphoreType.DMA((21,)), pltpu.SemaphoreType.DMA, pltpu.SemaphoreType.REGULAR,
        ],
        compiler_params=pltpu.CompilerParams(vmem_limit_bytes=110 * 1024 * 1024),
    )(c, A_shift_k.T, A_ssm_D,
      A_q.reshape(S, D), A_k.reshape(S, D), A_v.reshape(S, D), A_ssm_k,
      B_W_gate, B_W_up, B_W_down, w_mod, jnp.asarray(_FB), jnp.asarray(_GB))
    return out.reshape(1, S, D)
```
